```python
import jax
import jax.numpy as jnp

def _softmax(x, axis=-1):
    return jax.nn.softmax(x, axis=axis)
def _gelu(x):
    return jax.nn.gelu(x, approximate=True)
def _silu(x):
    return jax.nn.silu(x)
def _sigmoid(x):
    return jax.nn.sigmoid(x)
def _layernorm(x, axis=-1, eps=1e-5):
    m = jnp.mean(x, axis=axis, keepdims=True)
    v = jnp.var(x, axis=axis, keepdims=True)
    return (x - m) / jnp.sqrt(v + eps)
def _scatter_add(tgt, idx, src, axis=0):
    return tgt.at[idx].add(src)
def _segment_sum(src, seg, n):
    return jax.ops.segment_sum(src, seg, n)
class _Rng:
    def __init__(self, key):
        self._k = key
    def _next(self):
        self._k, sub = jax.random.split(self._k)
        return sub
    def normal(self, shape):
        return jax.random.normal(self._next(), shape, dtype=jnp.bfloat16)
    def randint(self, lo, hi, shape):
        return jax.random.randint(self._next(), shape, lo, hi, dtype=jnp.int32)
    def uniform(self, shape, lo=0.0, hi=1.0):
        return jax.random.uniform(self._next(), shape, jnp.bfloat16, lo, hi)
    def permutation(self, n):
        return jax.random.permutation(self._next(), n)


kernel_name = 'interleave_layers__sliding_local_dilated__mixer_token_mlp__prompt'

def setup_inputs():
    _rng = _Rng(jax.random.key(int.from_bytes(__import__("os").urandom(4), "little")))
    _w = (lambda a: (lambda t: t.astype(jnp.bfloat16) if jnp.issubdtype(t.dtype, jnp.floating) else t)(jnp.asarray(a)))
    def _A_setup():
        B, S, D = 1, 2048, 1024
        return {
            "x": _w((lambda *s: _rng.normal(s) * 0.05)(B, S, D)),
            "wqkv": _w((lambda *s: _rng.normal(s) * 0.05)(D, 3 * D)),
            "wo": _w((lambda *s: _rng.normal(s) * 0.05)(D, D)),
        }
    _A_in = _A_setup()

    def _B_setup():
        B, S, D, F = 1, 2048, 1024, 3584
        return {
            "x": _w((lambda *s: _rng.normal(s) * 0.05)(B, S, D)),
            "w1": _w((lambda *s: _rng.normal(s) * 0.05)(S, F) * (S ** -0.5)),
            "b1": _w((lambda *s: _rng.normal(s) * 0.05)(F) * 0.02),
            "w2": _w((lambda *s: _rng.normal(s) * 0.05)(F, S) * (F ** -0.5)),
            "b2": _w((lambda *s: _rng.normal(s) * 0.05)(S) * 0.02),
        }
    _B_in = _B_setup()

    return {
        "A_x": _A_in["x"],
        "A_wqkv": _A_in["wqkv"],
        "A_wo": _A_in["wo"],
        "B_x": _B_in["x"],
        "B_w1": _B_in["w1"],
        "B_b1": _B_in["b1"],
        "B_w2": _B_in["w2"],
        "B_b2": _B_in["b2"],
    }

def reference(A_x, A_wqkv, A_wo, B_x, B_w1, B_b1, B_w2, B_b2):
    def _A_ref(x, wqkv, wo):
        B, S, D = x.shape
        H = 32; Dh = D // H
        W, dil = 8, 2
        qkv = (lambda x, *d: x.transpose(*d))((x @ wqkv).reshape(B, S, 3, H, Dh), 2, 0, 3, 1, 4)
        q, k, v = qkv[0], qkv[1], qkv[2]
        scale = Dh ** -0.5
        pos = jnp.arange(S)
        off = jnp.arange(W) * dil
        idx = pos[:, None] - off[None, :]
        mask = idx >= 0
        idx_c = jnp.where(mask, idx, 0).reshape(-1)
        kg = k[:, :, idx_c, :].reshape(B, H, S, W, Dh)
        vg = v[:, :, idx_c, :].reshape(B, H, S, W, Dh)
        logits = jnp.einsum("bhsd,bhswd->bhsw", q, kg) * scale
        logits = jnp.where(mask[None, None, :, :], logits, -1e9)
        attn = _softmax(logits, axis=-1)
        o = jnp.einsum("bhsw,bhswd->bhsd", attn, vg)
        return (lambda x, *d: x.transpose(*d))(o, 0, 2, 1, 3).reshape(B, S, D) @ wo

    def _B_ref(x, w1, b1, w2, b2):
        B, S, D = x.shape
        h = _layernorm(x, axis=-1)
        u = jnp.einsum("bsd,sf->bdf", h, w1) + b1
        u = _gelu(u)
        y = jnp.einsum("bdf,fs->bds", u, w2) + b2
        return (lambda x, *d: x.transpose(*d))(y, 0, 2, 1)

    x = A_x
    x = x + _A_ref(_layernorm(x, axis=-1), A_wqkv, A_wo)
    x = x + _B_ref(_layernorm(x, axis=-1), B_w1, B_b1, B_w2, B_b2)
    x = x + _A_ref(_layernorm(x, axis=-1), A_wqkv, A_wo)
    x = x + _B_ref(_layernorm(x, axis=-1), B_w1, B_b1, B_w2, B_b2)
    return x
```

```python
import math

import jax
import jax.numpy as jnp
from jax import lax
import jax.experimental.pallas as pl
import jax.experimental.pallas.tpu as pltpu

S, D, F = 2048, 1024, 3584
H, DH, W, DIL = 32, 32, 8, 2
BS = 256
NB = S // BS
RT = 16
HALO = 16
FC = 512
NC = D // 128
EPS = 1e-5
F32, BF16 = jnp.float32, jnp.bfloat16


def _ln(x):
    m = jnp.mean(x, axis=-1, keepdims=True)
    c = x - m
    v = jnp.mean(c * c, axis=-1, keepdims=True)
    return c * lax.rsqrt(v + EPS)


def _gelu(x):
    c = math.sqrt(2.0 / math.pi)
    return (0.5 * x) * (1.0 + jnp.tanh(x * (c + (c * 0.044715) * (x * x))))


def _kernel(x_hbm, wqkv_hbm, wo_hbm, w1_hbm, b1_ref, w2_hbm, b2_ref, out_hbm,
            xin, wqkv, wo, w1, w2, xs, qs, ks, vs, os_, hT, u, tmp, ob, sems):
    def rows(i):
        return pl.ds(pl.multiple_of(i * BS, BS), BS)

    def col(g):
        return pl.ds(g * D, D)

    cp_x0 = pltpu.make_async_copy(x_hbm.at[pl.ds(0, BS)], xin.at[pl.ds(0, BS)], sems.at[0])
    cp_w = [pltpu.make_async_copy(wqkv_hbm.at[:, col(g)], wqkv.at[:, col(g)], sems.at[1 + g])
            for g in range(3)]
    cp_x1 = pltpu.make_async_copy(x_hbm.at[pl.ds(BS, S - BS)], xin.at[pl.ds(BS, S - BS)], sems.at[4])
    cp_wo = pltpu.make_async_copy(wo_hbm, wo, sems.at[5])
    cp_w1 = pltpu.make_async_copy(w1_hbm, w1, sems.at[6])
    cp_w2 = pltpu.make_async_copy(w2_hbm, w2, sems.at[7])

    def cp_out(i):
        return pltpu.make_async_copy(ob.at[rows(i)], out_hbm.at[rows(i)], sems.at[8])

    cp_w[0].start()
    cp_x0.start()
    cp_w[1].start()
    cp_w[2].start()
    cp_wo.start()
    cp_x1.start()

    ks[:, pl.ds(0, HALO), :] = jnp.zeros((NC, HALO, 128), F32)
    vs[:, pl.ds(0, HALO), :] = jnp.zeros((NC, HALO, 128), F32)

    for g in range(3):
        cp_w[g].wait()
        wi = pltpu.bitcast(wqkv[:, col(g)], jnp.int32)
        for t in range(4):
            tmp[t] = wi[t * 128:(t + 1) * 128, :].T
        for t in range(4):
            for c in range(NC):
                blk = jnp.concatenate(
                    [tmp[t, pl.ds(4 * c + j, H, stride=DH), :] for j in range(4)], axis=0)
                wqkv[pl.ds(t * 256, 256), pl.ds(g * D + c * 128, 128)] = pltpu.bitcast(blk.T, BF16)
        if g == 2:
            cp_w1.start()
            cp_w2.start()
    cp_wo.wait()
    for t in range(2):
        for c in range(4):
            tmp[c] = pltpu.bitcast(wo[:, pl.ds((t * 4 + c) * 128, 128)].astype(F32), jnp.int32)
        for c in range(4):
            blk = jnp.concatenate(
                [tmp[c, pl.ds(d, H, stride=DH), :] for d in range(DH)], axis=0)
            wo[:, pl.ds((t * 4 + c) * 128, 128)] = pltpu.bitcast(blk, F32).astype(BF16)

    def mix_out(i):
        y = jnp.dot(u[...], w2[:, rows(i)], preferred_element_type=F32) + b2_ref[:, rows(i)]
        return xs[rows(i), :] + y.T

    def s_qkv(i, first):
        x = xin[rows(i), :].astype(F32) if first else mix_out(i)
        xs[rows(i), :] = x
        xn = _ln(x).astype(BF16)
        hrows = pl.ds(pl.multiple_of(i * BS + HALO, HALO), BS)
        for g, (dst, r) in enumerate(((qs, rows(i)), (ks, hrows), (vs, hrows))):
            y = jnp.dot(xn, wqkv[:, col(g)], preferred_element_type=F32)
            for c in range(NC):
                dst[c, r, :] = y[:, c * 128:(c + 1) * 128]

    def s_att(i):
        sc = DH ** -0.5
        for t in range(BS // RT):
            r0 = i * BS + t * RT
            acc = [None] * W
            for c in range(NC):
                q = qs[c, pl.ds(pl.multiple_of(r0, RT), RT), :]
                for w in range(W):
                    p = q * ks[c, pl.ds(r0 + (HALO - DIL * w), RT), :]
                    acc[w] = p if c == 0 else acc[w] + p
            lg = []
            for w in range(W):
                a = acc[w] + pltpu.roll(acc[w], 64, 1)
                a = (a + pltpu.roll(a, 32, 1)) * sc
                if t == 0 and w > 0:
                    pos = r0 + lax.broadcasted_iota(jnp.int32, (RT, 128), 0)
                    a = jnp.where(pos >= DIL * w, a, -1e9)
                lg.append(a)
            m = lg[0]
            for w in range(1, W):
                m = jnp.maximum(m, lg[w])
            e = [jnp.exp(a - m) for a in lg]
            den = e[0]
            for w in range(1, W):
                den = den + e[w]
            inv = 1.0 / den
            e = [a * inv for a in e]
            for c in range(NC):
                o = None
                for w in range(W):
                    p = e[w] * vs[c, pl.ds(r0 + (HALO - DIL * w), RT), :]
                    o = p if o is None else o + p
                os_[pl.ds(pl.multiple_of(r0, RT), RT), pl.ds(c * 128, 128)] = o.astype(BF16)

    def s_out(i):
        x = xs[rows(i), :] + jnp.dot(os_[rows(i), :], wo[...], preferred_element_type=F32)
        xs[rows(i), :] = x
        hT[:, rows(i)] = _ln(_ln(x)).T.astype(BF16)

    def phase_a(first):
        s_qkv(0, first)

        def body(i, _):
            s_qkv(i + 1, first)
            s_att(i)
            s_out(i)

        lax.fori_loop(0, NB - 1, body, None)
        s_att(NB - 1)
        s_out(NB - 1)

    def phase_b():
        def body(j, _):
            fc = pl.ds(pl.multiple_of(j * FC, FC), FC)
            a = jnp.dot(hT[...], w1[:, fc], preferred_element_type=F32) + b1_ref[:, fc]
            u[:, fc] = _gelu(a).astype(BF16)

        lax.fori_loop(0, F // FC, body, None)

    cp_x0.wait()
    cp_x1.wait()
    phase_a(True)
    cp_w1.wait()
    phase_b()
    cp_w2.wait()
    phase_a(False)
    phase_b()

    def fin(i, _):
        ob[rows(i), :] = mix_out(i).astype(BF16)
        cp_out(i).start()

    lax.fori_loop(0, NB, fin, None)
    pltpu.make_async_copy(ob, out_hbm, sems.at[8]).wait()


@jax.jit
def pallas_interleave_layers__sliding_local_dilated__mixer_token_mlp__prompt_kernel(
    A_x, A_wqkv, A_wo, B_x, B_w1, B_b1, B_w2, B_b2,
):
    del B_x
    hbm = pl.BlockSpec(memory_space=pl.ANY)
    vm = pl.BlockSpec(memory_space=pltpu.VMEM)
    out = pl.pallas_call(
        _kernel,
        in_specs=[hbm, hbm, hbm, hbm, vm, hbm, vm],
        out_specs=hbm,
        out_shape=jax.ShapeDtypeStruct((S, D), BF16),
        scratch_shapes=[
            pltpu.VMEM((S, D), BF16),
            pltpu.VMEM((D, 3 * D), BF16),
            pltpu.VMEM((D, D), BF16),
            pltpu.VMEM((S, F), BF16),
            pltpu.VMEM((F, S), BF16),
            pltpu.VMEM((S, D), F32),
            pltpu.VMEM((NC, S, 128), F32),
            pltpu.VMEM((NC, S + HALO, 128), F32),
            pltpu.VMEM((NC, S + HALO, 128), F32),
            pltpu.VMEM((S, D), BF16),
            pltpu.VMEM((D, S), BF16),
            pltpu.VMEM((D, F), BF16),
            pltpu.VMEM((4, D, 128), jnp.int32),
            pltpu.VMEM((S, D), BF16),
            pltpu.SemaphoreType.DMA((9,)),
        ],
        compiler_params=pltpu.CompilerParams(vmem_limit_bytes=120 * 1024 * 1024),
    )(A_x.reshape(S, D), A_wqkv, A_wo, B_w1, B_b1.reshape(1, F).astype(F32), B_w2,
      B_b2.reshape(1, S).astype(F32))
    return out.reshape(1, S, D)
```

```python
import math

import jax
import jax.numpy as jnp
from jax import lax
import jax.experimental.pallas as pl
import jax.experimental.pallas.tpu as pltpu

S, D, F = 2048, 1024, 3584
H, DH, W, DIL = 32, 32, 8, 2
BS = 256
NB = S // BS
RT = 16
HALO = 16
FC = 512
NC = D // 128
EPS = 1e-5
F32, BF16 = jnp.float32, jnp.bfloat16


def _ln(x):
    m = jnp.mean(x, axis=-1, keepdims=True)
    c = x - m
    v = jnp.mean(c * c, axis=-1, keepdims=True)
    return c * lax.rsqrt(v + EPS)


def _gelu(x):
    c = math.sqrt(2.0 / math.pi)
    return (0.5 * x) * (1.0 + jnp.tanh(x * (c + (c * 0.044715) * (x * x))))


def _kernel(x_hbm, wqkv_hbm, wo_hbm, w1_hbm, b1_in, w2_hbm, b2_in, out_hbm,
            xin, wqkv, wo, w1, w2, xs, qs, ks, vs, os_, hT, u, tmp, ob, b1_ref, b2_ref, sems):
    def rows(i):
        return pl.ds(pl.multiple_of(i * BS, BS), BS)

    def col(g):
        return pl.ds(g * D, D)

    cp_x0 = pltpu.make_async_copy(x_hbm.at[pl.ds(0, 2 * BS)], xin.at[pl.ds(0, 2 * BS)], sems.at[0])
    cp_w = [pltpu.make_async_copy(wqkv_hbm.at[:, col(g)], wqkv.at[:, col(g)], sems.at[1 + g])
            for g in range(3)]
    cp_x1 = pltpu.make_async_copy(x_hbm.at[pl.ds(2 * BS, S - 2 * BS)], xin.at[pl.ds(2 * BS, S - 2 * BS)], sems.at[4])
    cp_wo = pltpu.make_async_copy(wo_hbm, wo, sems.at[5])
    cp_w1 = pltpu.make_async_copy(w1_hbm, w1, sems.at[6])
    cp_w2 = pltpu.make_async_copy(w2_hbm, w2, sems.at[7])

    def cp_out(i):
        return pltpu.make_async_copy(ob.at[rows(i)], out_hbm.at[rows(i)], sems.at[8])

    cp_w[1].start()
    cp_x0.start()
    cp_w[2].start()
    cp_w[0].start()
    cp_wo.start()
    cp_x1.start()

    ks[:, pl.ds(0, HALO), :] = jnp.zeros((NC, HALO, 128), F32)
    vs[:, pl.ds(0, HALO), :] = jnp.zeros((NC, HALO, 128), F32)

    def put(t, v):
        for h in range(H):
            tmp[t, pl.ds(h * (DH + 1), DH), :] = v[h * DH:(h + 1) * DH]

    def perm_cols(g):
        cp_w[g].wait()
        wi = pltpu.bitcast(wqkv[:, col(g)], jnp.int32)
        for t in range(4):
            put(t, wi[t * 128:(t + 1) * 128, :].T)
        for t in range(4):
            for c in range(NC):
                blk = jnp.concatenate(
                    [tmp[t, pl.ds(4 * c + j, H, stride=DH + 1), :] for j in range(4)], axis=0)
                wqkv[pl.ds(t * 256, 256), pl.ds(g * D + c * 128, 128)] = pltpu.bitcast(blk.T, BF16)

    def perm_wo():
      for t in range(2):
        for c in range(4):
            put(c, pltpu.bitcast(wo[:, pl.ds((t * 4 + c) * 128, 128)].astype(F32), jnp.int32))
        for c in range(4):
            blk = jnp.concatenate(
                [tmp[c, pl.ds(d, H, stride=DH + 1), :] for d in range(DH)], axis=0)
            wo[:, pl.ds((t * 4 + c) * 128, 128)] = pltpu.bitcast(blk, F32).astype(BF16)

    def mix_out(i):
        y = jnp.dot(u[...], w2[:, rows(i)], preferred_element_type=F32) + b2_ref[:, rows(i)]
        return xs[rows(i), :] + y.T

    def s_pre(i, first):
        return xin[rows(i), :].astype(F32) if first else mix_out(i)

    def s_qkv(i, x):
        xs[rows(i), :] = x
        xn = _ln(x).astype(BF16)
        for g in range(3):
            proj(xn, g, i * BS)

    def proj(xn, g, r0):
        r = pl.ds(pl.multiple_of(r0 + (HALO if g else 0), HALO), xn.shape[0])
        y = jnp.dot(xn, wqkv[:, col(g)], preferred_element_type=F32)
        for c in range(NC):
            (qs, ks, vs)[g][c, r, :] = y[:, c * 128:(c + 1) * 128]

    def s_att(i):
        sc = DH ** -0.5
        for t in range(BS // RT):
            r0 = i * BS + t * RT
            acc = [None] * W
            for c in range(NC):
                q = qs[c, pl.ds(pl.multiple_of(r0, RT), RT), :]
                for w in range(W):
                    p = q * ks[c, pl.ds(r0 + (HALO - DIL * w), RT), :]
                    acc[w] = p if c == 0 else acc[w] + p
            lg = []
            for w in range(W):
                a = acc[w] + pltpu.roll(acc[w], 64, 1)
                a = (a + pltpu.roll(a, 32, 1)) * sc
                if t == 0 and w > 0:
                    pos = r0 + lax.broadcasted_iota(jnp.int32, (RT, 128), 0)
                    a = jnp.where(pos >= DIL * w, a, -1e9)
                lg.append(a)
            m = lg[0]
            for w in range(1, W):
                m = jnp.maximum(m, lg[w])
            e = [jnp.exp(a - m) for a in lg]
            den = e[0]
            for w in range(1, W):
                den = den + e[w]
            inv = 1.0 / den
            e = [a * inv for a in e]
            for c in range(NC):
                o = None
                for w in range(W):
                    p = e[w] * vs[c, pl.ds(r0 + (HALO - DIL * w), RT), :]
                    o = p if o is None else o + p
                os_[pl.ds(pl.multiple_of(r0, RT), RT), pl.ds(c * 128, 128)] = o.astype(BF16)

    def s_out(i):
        x = xs[rows(i), :] + jnp.dot(os_[rows(i), :], wo[...], preferred_element_type=F32)
        xs[rows(i), :] = x
        hT[:, rows(i)] = _ln(_ln(x)).T.astype(BF16)

    def phase_a(first):
        if first:
            b1_ref[...] = b1_in[...].astype(F32).reshape(1, F)
            b2_ref[...] = b2_in[...].astype(F32).reshape(1, S)
            perm_cols(1)
            cp_x0.wait()
            x = xin[pl.ds(0, 2 * BS), :].astype(F32)
            xs[pl.ds(0, 2 * BS), :] = x
            xn = _ln(x).astype(BF16)
            perm_cols(2)
            proj(xn, 1, 0)
            perm_cols(0)
            proj(xn, 2, 0)
            cp_wo.wait()
            cp_w1.start()
            cp_w2.start()
            perm_wo()
            proj(xn[:BS], 0, 0)
            s_att(0)
            proj(xn[BS:], 0, BS)
            cp_x1.wait()
        else:
            x = s_pre(0, first)
            x1 = s_pre(1, first)
            s_qkv(0, x)
            s_att(0)
            s_qkv(1, x1)

        def body(i, _):
            x = s_pre(i + 1, first)
            s_out(i - 1)
            s_att(i)
            s_qkv(i + 1, x)

        lax.fori_loop(1, NB - 1, body, None)
        s_out(NB - 2)
        s_att(NB - 1)
        s_out(NB - 1)

    def phase_b():
        def body(j, _):
            fc = pl.ds(pl.multiple_of(j * FC, FC), FC)
            a = jnp.dot(hT[...], w1[:, fc], preferred_element_type=F32) + b1_ref[:, fc]
            u[:, fc] = _gelu(a).astype(BF16)

        lax.fori_loop(0, F // FC, body, None)

    phase_a(True)
    cp_w1.wait()
    phase_b()
    cp_w2.wait()
    phase_a(False)
    phase_b()

    def fin(i, _):
        ob[rows(i), :] = mix_out(i).astype(BF16)
        cp_out(i).start()

    lax.fori_loop(0, NB, fin, None)
    pltpu.make_async_copy(ob, out_hbm, sems.at[8]).wait()


@jax.jit
def pallas_interleave_layers__sliding_local_dilated__mixer_token_mlp__prompt_kernel(
    A_x, A_wqkv, A_wo, B_x, B_w1, B_b1, B_w2, B_b2,
):
    del B_x
    hbm = pl.BlockSpec(memory_space=pl.ANY)
    vm = pl.BlockSpec(memory_space=pltpu.VMEM)
    out = pl.pallas_call(
        _kernel,
        in_specs=[hbm, hbm, hbm, hbm, vm, hbm, vm],
        out_specs=hbm,
        out_shape=jax.ShapeDtypeStruct((S, D), BF16),
        scratch_shapes=[
            pltpu.VMEM((S, D), BF16),
            pltpu.VMEM((D, 3 * D), BF16),
            pltpu.VMEM((D, D), BF16),
            pltpu.VMEM((S, F), BF16),
            pltpu.VMEM((F, S), BF16),
            pltpu.VMEM((S, D), F32),
            pltpu.VMEM((NC, S, 128), F32),
            pltpu.VMEM((NC, S + HALO, 128), F32),
            pltpu.VMEM((NC, S + HALO, 128), F32),
            pltpu.VMEM((S, D), BF16),
            pltpu.VMEM((D, S), BF16),
            pltpu.VMEM((D, F), BF16),
            pltpu.VMEM((4, D + H, 128), jnp.int32),
            pltpu.VMEM((S, D), BF16),
            pltpu.VMEM((1, F), F32),
            pltpu.VMEM((1, S), F32),
            pltpu.SemaphoreType.DMA((9,)),
        ],
        compiler_params=pltpu.CompilerParams(vmem_limit_bytes=120 * 1024 * 1024),
    )(A_x.reshape(S, D), A_wqkv, A_wo, B_w1, B_b1, B_w2,
      B_b2)
    return out.reshape(1, S, D)
```
